```python
import jax
import jax.numpy as jnp

def _softmax(x, axis=-1):
    return jax.nn.softmax(x, axis=axis)
def _gelu(x):
    return jax.nn.gelu(x, approximate=True)
def _silu(x):
    return jax.nn.silu(x)
def _sigmoid(x):
    return jax.nn.sigmoid(x)
def _layernorm(x, axis=-1, eps=1e-5):
    m = jnp.mean(x, axis=axis, keepdims=True)
    v = jnp.var(x, axis=axis, keepdims=True)
    return (x - m) / jnp.sqrt(v + eps)
def _scatter_add(tgt, idx, src, axis=0):
    return tgt.at[idx].add(src)
def _segment_sum(src, seg, n):
    return jax.ops.segment_sum(src, seg, n)
class _Rng:
    def __init__(self, key):
        self._k = key
    def _next(self):
        self._k, sub = jax.random.split(self._k)
        return sub
    def normal(self, shape):
        return jax.random.normal(self._next(), shape, dtype=jnp.bfloat16)
    def randint(self, lo, hi, shape):
        return jax.random.randint(self._next(), shape, lo, hi, dtype=jnp.int32)
    def uniform(self, shape, lo=0.0, hi=1.0):
        return jax.random.uniform(self._next(), shape, jnp.bfloat16, lo, hi)
    def permutation(self, n):
        return jax.random.permutation(self._next(), n)


kernel_name = 'concat_heads__gqa_block_cached__compressed_kv_cla__decode'

def setup_inputs():
    _rng = _Rng(jax.random.key(int.from_bytes(__import__("os").urandom(4), "little")))
    _w = (lambda a: (lambda t: t.astype(jnp.bfloat16) if jnp.issubdtype(t.dtype, jnp.floating) else t)(jnp.asarray(a)))
    def _A_setup():
        B, Sq, D = 2, 1, 512
        Hq, Hkv, Sk, Dh = 32, 32, 8192, 128
        assert Hq % Hkv == 0, (Hq, Hkv)
        return {
            "x": _w((lambda *s: _rng.normal(s) * 0.05)(B, Sq, D)),
            "k_cache": _w((lambda *s: _rng.normal(s) * 0.05)(B, Hkv, Sk, Dh)),
            "v_cache": _w((lambda *s: _rng.normal(s) * 0.05)(B, Hkv, Sk, Dh)),
            "wq": _w((lambda *s: _rng.normal(s) * 0.05)(D, Hq * Dh) * (D ** -0.5)),
            "wo": _w((lambda *s: _rng.normal(s) * 0.05)(Hq * Dh, D) * ((Hq * Dh) ** -0.5)),
        }
    _A_in = _A_setup()

    def _B_setup():
        B, H, Sq, Sk, D, M = 2, 32, 1, 8192, 128, 512
        Dc = 4 * D
        return {
            "x": _w((lambda *s: _rng.normal(s) * 0.05)(B, Sq, M)),
            "c_kv": _w((lambda *s: _rng.normal(s) * 0.05)(B, Sk, Dc)),
            "w_q": _w((lambda *s: _rng.normal(s) * 0.05)(M, H, D) * (M ** -0.5)),
            "w_uk": _w((lambda *s: _rng.normal(s) * 0.05)(Dc, H, D) * (Dc ** -0.5)),
            "w_uv": _w((lambda *s: _rng.normal(s) * 0.05)(Dc, H, D) * (Dc ** -0.5)),
            "w_o": _w((lambda *s: _rng.normal(s) * 0.05)(H, D, M) * ((H * D) ** -0.5)),
        }
    _B_in = _B_setup()

    return {
        "A_x": _A_in["x"],
        "A_k_cache": _A_in["k_cache"],
        "A_v_cache": _A_in["v_cache"],
        "A_wq": _A_in["wq"],
        "A_wo": _A_in["wo"],
        "B_x": _B_in["x"],
        "B_c_kv": _B_in["c_kv"],
        "B_w_q": _B_in["w_q"],
        "B_w_uk": _B_in["w_uk"],
        "B_w_uv": _B_in["w_uv"],
        "B_w_o": _B_in["w_o"],
    }

def reference(A_x, A_k_cache, A_v_cache, A_wq, A_wo, B_x, B_c_kv, B_w_q, B_w_uk, B_w_uv, B_w_o):
    def _A_ref(x, k_cache, v_cache, wq, wo):
        B, Sq, D = x.shape
        Hq, Dh = 32, 128
        Hkv = k_cache.shape[1]
        rep = Hq // Hkv
        q = (lambda x, *d: x.transpose(*d))((x @ wq).reshape(B, Sq, Hq, Dh), 0, 2, 1, 3)
        k = jnp.repeat(k_cache, rep, axis=1)
        v = jnp.repeat(v_cache, rep, axis=1)
        scores = jnp.einsum("bhqd,bhkd->bhqk", q, k) * (Dh ** -0.5)
        p = _softmax(scores, axis=-1)
        o = jnp.einsum("bhqk,bhkd->bhqd", p, v)
        return (lambda x, *d: x.transpose(*d))(o, 0, 2, 1, 3).reshape(B, Sq, Hq * Dh) @ wo

    def _B_ref(x, c_kv, w_q, w_uk, w_uv, w_o):
        B, Sq, M = x.shape[0], x.shape[1], x.shape[2]
        Sk = c_kv.shape[1]
        H, D = w_q.shape[1], w_q.shape[2]
        q = jnp.einsum("bqm,mhd->bhqd", x, w_q)
        k = jnp.einsum("bkc,chd->bhkd", c_kv, w_uk)
        v = jnp.einsum("bkc,chd->bhkd", c_kv, w_uv)
        scores = jnp.einsum("bhqd,bhkd->bhqk", q, k) * (D ** -0.5)
        off = Sk - Sq
        qi = jnp.arange(Sq)[:, None]
        kj = jnp.arange(Sk)[None, :]
        cmask = kj <= (qi + off)
        scores = jnp.where(cmask[None, None], scores, -1e9)
        p = _softmax(scores, axis=-1)
        ctx = jnp.einsum("bhqk,bhkd->bhqd", p, v)
        return jnp.einsum("bhqd,hdm->bqm", ctx, w_o)

    a = _A_ref(A_x, A_k_cache, A_v_cache, A_wq, A_wo)
    b = _B_ref(B_x, B_c_kv, B_w_q, B_w_uk, B_w_uv, B_w_o)
    return jnp.concatenate([a, b], axis=-1)
```

```python
import jax
import jax.numpy as jnp
import jax.experimental.pallas as pl
import jax.experimental.pallas.tpu as pltpu

_NT = (((1,), (1,)), ((), ()))
_NN = (((1,), (0,)), ((), ()))
_TN = (((0,), (0,)), ((), ()))
_LOG2E = 1.4426950408889634

TILE = 128
RING = 3
LOOKAHEAD = 2
CH = 64


def _dot(a, b, dims):
    return jax.lax.dot_general(a, b, dims, preferred_element_type=jnp.float32)


def _build_kernel(NB, H, S, D, DM, DC, ckv_big_rows, phases):
    NH = NB * H
    NT_S = S // TILE
    scale_log2e = (D ** -0.5) * _LOG2E
    assert NB == 2 and NB * H <= 128 and D == 128

    def kernel(xa_hbm, k_hbm, v_hbm, wq_hbm, wo_hbm, xb_hbm, ckv_hbm, wqb_hbm, wuk_hbm, wuv_hbm, wob_hbm,
               out_ref,
               xa_v, xb_v, wq_v, wo_v, ckv_v, wqb_v, wuk_v, wuv_v, wob_v,
               kbuf, vbuf, sbuf, qa_s, xbc_s, t_s, ql_s, cl_s,
               sems, ksem, vsem):
        SEM_XA, SEM_XB, SEM_WQ, SEM_WO, SEM_CKV_A, SEM_CKV_B, SEM_CKV_C, SEM_WQB, SEM_WUK, SEM_WUV, SEM_WOB = range(11)

        def cp(src, dst, sem):
            return pltpu.make_async_copy(src, dst, sem)

        def issue_pairs(n, mk0, mk1, unroll=4):
            assert n % unroll == 0

            def body(i, c):
                for u in range(unroll):
                    mk0(i * unroll + u).start(priority=0)
                    mk1(i * unroll + u).start(priority=1)
                return c
            jax.lax.fori_loop(0, n // unroll, body, 0)

        def rows_chunk(hbm, vmem, sem, nrows, base=0):
            def mk(i):
                r = pl.ds(pl.multiple_of(base + i * nrows, nrows), nrows)
                return cp(hbm.at[r, :], vmem.at[r, :], sems.at[sem])
            return mk

        cp(xb_hbm, xb_v, sems.at[SEM_XB]).start()
        cp(xa_hbm, xa_v, sems.at[SEM_XA]).start()
        n_w = (DM * H) // TILE
        issue_pairs(n_w, rows_chunk(wqb_hbm, wqb_v, SEM_WQB, TILE), rows_chunk(wuk_hbm, wuk_v, SEM_WUK, TILE))

        ckv_a = cp(ckv_hbm.at[pl.ds(0, ckv_big_rows), :], ckv_v.at[pl.ds(0, ckv_big_rows), :], sems.at[SEM_CKV_A])
        ckv_a.start(priority=1)

        cp(xb_hbm, xb_v, sems.at[SEM_XB]).wait()
        cp(wqb_hbm, wqb_v, sems.at[SEM_WQB]).wait()

        xbf = xb_v[...].astype(jnp.float32)
        for b in range(NB):
            xbc_s[b] = jnp.broadcast_to(xbf[b:b + 1, :], (128, DM)).T

        def b1_body(m, carry):
            a0, a1 = carry
            w = wqb_v[pl.ds(pl.multiple_of(m * H, H), H), :].astype(jnp.float32)
            return a0 + w * xbc_s[0, pl.ds(m, 1), :], a1 + w * xbc_s[1, pl.ds(m, 1), :]
        z = jnp.zeros((H, D), jnp.float32)
        q0, q1 = jax.lax.fori_loop(0, DM, b1_body, (z, z), unroll=8)
        qm = jnp.concatenate([q0, q1, jnp.zeros((128 - NB * H, D), jnp.float32)], axis=0).astype(jnp.bfloat16)

        cp(wuk_hbm, wuk_v, sems.at[SEM_WUK]).wait()
        rows = jax.lax.broadcasted_iota(jnp.int32, (CH * H, 128), 0)
        lanes = jax.lax.broadcasted_iota(jnp.int32, (CH * H, 128), 1)
        mask2 = (rows % H) == (lanes % H)

        def b2_chunk(i, c):
            w = wuk_v[pl.ds(pl.multiple_of(i * CH * H, CH * H), CH * H), :]
            o = _dot(w, qm, _NT)
            o = jnp.where(mask2, o, 0.0).reshape(CH, H, 128)
            t_s[pl.ds(pl.multiple_of(i * CH, CH), CH), :] = jnp.sum(o, axis=1)
            return c
        jax.lax.fori_loop(0, DC // CH, b2_chunk, 0)
        ql_s[...] = t_s[...].T

        rest = NB * S - ckv_big_rows
        CR = 32
        half = rest // 2
        issue_pairs(half // CR,
                    rows_chunk(ckv_hbm, ckv_v, SEM_CKV_B, CR, ckv_big_rows),
                    rows_chunk(ckv_hbm, ckv_v, SEM_CKV_C, CR, ckv_big_rows + half))
        cp(wuv_hbm, wuv_v, sems.at[SEM_WUV]).start(priority=1)
        cp(wob_hbm, wob_v, sems.at[SEM_WOB]).start(priority=1)

        ckv_a.wait()
        cp(ckv_hbm.at[pl.ds(ckv_big_rows, half), :], ckv_v.at[pl.ds(ckv_big_rows, half), :], sems.at[SEM_CKV_B]).wait()
        cp(ckv_hbm.at[pl.ds(ckv_big_rows + half, half), :], ckv_v.at[pl.ds(ckv_big_rows + half, half), :],
           sems.at[SEM_CKV_C]).wait()
        for b in range(NB):
            qlb = ql_s[pl.ds(b * H, H), :].astype(jnp.bfloat16)
            c = ckv_v[pl.ds(b * S, S), :]
            s = _dot(qlb, c, _NT)
            m = jnp.max(s, axis=1, keepdims=True)
            p = jnp.exp2((s - m) * scale_log2e)
            l = jnp.sum(p, axis=1, keepdims=True)
            cl = _dot(p.astype(jnp.bfloat16), c, _NN)
            cl_s[pl.ds(b * H, H), :] = cl / l
        cl_s[pl.ds(NB * H, 128 - NB * H), :] = jnp.zeros((128 - NB * H, DC), jnp.float32)

        def wq_chunk(i):
            ncb = wq_hbm.shape[1] // 2048
            r = pl.ds(pl.multiple_of((i // ncb) * 8, 8), 8)
            c = pl.ds(pl.multiple_of((i % ncb) * 2048, 2048), 2048)
            return cp(wq_hbm.at[r, c], wq_v.at[r, c], sems.at[SEM_WQ])
        n_wq = (wq_hbm.shape[0] // 8) * (wq_hbm.shape[1] // 2048)
        issue_pairs(n_wq, wq_chunk, rows_chunk(wo_hbm, wo_v, SEM_WO, 32))

        def k_big(h, slot):
            return cp(k_hbm.at[pl.ds(h * S, S), :], kbuf.at[slot], ksem.at[slot])

        def v_big(h, slot):
            return cp(v_hbm.at[pl.ds(h * S, S), :], vbuf.at[slot], vsem.at[slot])
        k_big(0, 0).start(priority=1)
        v_big(0, 0).start(priority=1)

        cp(wuv_hbm, wuv_v, sems.at[SEM_WUV]).wait()
        t_s[...] = cl_s[...].T
        rows3 = jax.lax.broadcasted_iota(jnp.int32, (CH, H, 128), 1)
        lanes3 = jax.lax.broadcasted_iota(jnp.int32, (CH, H, 128), 2)
        mask5 = rows3 == (lanes3 % H)

        def b5_chunk(i, acc):
            yt = t_s[pl.ds(pl.multiple_of(i * CH, CH), CH), :]
            zz = jnp.where(mask5, jnp.broadcast_to(yt[:, None, :], (CH, H, 128)), 0.0)
            zz = zz.reshape(CH * H, 128).astype(jnp.bfloat16)
            w = wuv_v[pl.ds(pl.multiple_of(i * CH * H, CH * H), CH * H), :]
            return acc + _dot(zz, w, _TN)
        ctx = jax.lax.fori_loop(0, DC // CH, b5_chunk, jnp.zeros((128, D), jnp.float32))

        cp(wob_hbm, wob_v, sems.at[SEM_WOB]).wait()
        rows8 = jax.lax.broadcasted_iota(jnp.int32, (8, D), 0)
        out_b = jnp.zeros((8, DM), jnp.float32)
        for hh in range(H):
            r0 = jnp.broadcast_to(ctx[hh:hh + 1, :], (8, D))
            r1 = jnp.broadcast_to(ctx[H + hh:H + hh + 1, :], (8, D))
            lhs = jnp.where(rows8 == 0, r0, jnp.where(rows8 == 1, r1, 0.0)).astype(jnp.bfloat16)
            out_b = out_b + _dot(lhs, wob_v[pl.ds(hh * D, D), :], _NN)
        out_ref[:, pl.ds(DM, DM)] = out_b[0:NB].astype(out_ref.dtype)

        cp(xa_hbm, xa_v, sems.at[SEM_XA]).wait()
        cp(wq_hbm, wq_v, sems.at[SEM_WQ]).wait()
        xaf = xa_v[...].astype(jnp.float32)
        rows_x = jax.lax.broadcasted_iota(jnp.int32, (8, DM), 0)
        xa8 = jnp.where(rows_x == 0, jnp.broadcast_to(xaf[0:1], (8, DM)),
                        jnp.where(rows_x == 1, jnp.broadcast_to(xaf[1:2], (8, DM)), 0.0)).astype(jnp.bfloat16)
        qa = _dot(xa8, wq_v[...], _NN).astype(jnp.bfloat16).astype(jnp.float32)
        for b in range(NB):
            for hh in range(H):
                qa_s[pl.ds(b * H + hh, 1), :] = qa[b:b + 1, hh * D:(hh + 1) * D]

        def start_pair(h, j):
            slot = h % RING
            r_src = pl.ds(pl.multiple_of(h * S + j * TILE, TILE), TILE)
            r_dst = pl.ds(j * TILE, TILE)
            cp(k_hbm.at[r_src, :], kbuf.at[slot, r_dst, :], ksem.at[slot]).start(priority=0)
            cp(v_hbm.at[r_src, :], vbuf.at[slot, r_dst, :], vsem.at[slot]).start(priority=1)

        def get_q(h):
            return jnp.broadcast_to(qa_s[pl.ds(h, 1), :], (8, D)).astype(jnp.bfloat16)

        def step(h, carry, do_dma, do_qk, do_pv):
            m_h, out_a = carry
            if do_pv:
                v_big(0, h % RING).wait()
            if do_qk:
                k_big(0, (h + 1) % RING).wait()
                q1 = get_q(h + 1)
            ks = (h + 1) % RING
            vs = h % RING
            sw = (h + 1) % 2
            sr = h % 2
            mrun = jnp.full((8, TILE), -jnp.inf, jnp.float32)
            lrun = jnp.zeros((8, TILE), jnp.float32)
            acc = jnp.zeros((8, D), jnp.float32)
            for j in range(NT_S):
                if do_dma:
                    start_pair(h + LOOKAHEAD, j)
                col = pl.ds(j * TILE, TILE)
                if do_pv:
                    p = jnp.exp2((sbuf[sr, :, col] - m_h) * scale_log2e)
                    lrun = lrun + p
                    acc = acc + _dot(p.astype(jnp.bfloat16), vbuf[vs, col, :], _NN)
                if do_qk:
                    s = _dot(q1, kbuf[ks, col, :], _NT)
                    sbuf[sw, :, col] = s
                    mrun = jnp.maximum(mrun, s)
            if do_pv:
                l = jnp.sum(lrun, axis=1, keepdims=True)
                o = (acc / l).astype(jnp.bfloat16).astype(jnp.float32)
                o = jnp.where(rows8 == h // H, o, 0.0).astype(jnp.bfloat16)
                r = pl.ds(pl.multiple_of((h % H) * D, D), D)
                out_a = out_a + _dot(o, wo_v[r, :], _NN)
            m_next = jnp.max(mrun, axis=1, keepdims=True) if do_qk else m_h
            return m_next, out_a

        cp(wo_hbm, wo_v, sems.at[SEM_WO]).wait()
        carry = (jnp.zeros((8, 1), jnp.float32), jnp.zeros((8, DM), jnp.float32))
        carry = step(-1, carry, True, True, False)
        carry = jax.lax.fori_loop(0, NH - LOOKAHEAD, lambda h, c: step(h, c, True, True, True), carry)
        for h in range(NH - LOOKAHEAD, NH):
            carry = step(h, carry, False, h + 1 < NH, True)
        out_ref[:, pl.ds(0, DM)] = carry[1][0:NB].astype(out_ref.dtype)

    return kernel


def _make_call(NB, H, S, D, DM, DC, ckv_big_rows=4096):
    NH = NB * H
    bf = jnp.bfloat16
    f32 = jnp.float32
    kernel = _build_kernel(NB, H, S, D, DM, DC, ckv_big_rows, None)
    any_spec = pl.BlockSpec(memory_space=pl.ANY)
    scratch = [
        pltpu.VMEM((NB, DM), bf), pltpu.VMEM((NB, DM), bf),
        pltpu.VMEM((DM, H * D), bf), pltpu.VMEM((H * D, DM), bf),
        pltpu.VMEM((NB * S, DC), bf),
        pltpu.VMEM((DM * H, D), bf), pltpu.VMEM((DC * H, D), bf), pltpu.VMEM((DC * H, D), bf),
        pltpu.VMEM((H * D, DM), bf),
        pltpu.VMEM((RING, S, D), bf), pltpu.VMEM((RING, S, D), bf),
        pltpu.VMEM((2, 8, S), f32),
        pltpu.VMEM((NH, D), f32),
        pltpu.VMEM((NB, DM, 128), f32),
        pltpu.VMEM((DC, 128), f32), pltpu.VMEM((128, DC), f32), pltpu.VMEM((128, DC), f32),
        pltpu.SemaphoreType.DMA((11,)), pltpu.SemaphoreType.DMA((RING,)), pltpu.SemaphoreType.DMA((RING,)),
    ]
    return pl.pallas_call(
        kernel,
        out_shape=jax.ShapeDtypeStruct((NB, 2 * DM), bf),
        in_specs=[any_spec] * 11,
        out_specs=pl.BlockSpec(memory_space=pltpu.VMEM),
        scratch_shapes=scratch,
        compiler_params=pltpu.CompilerParams(vmem_limit_bytes=100 * 2**20),
    )


@jax.jit
def pallas_concat_heads__gqa_block_cached__compressed_kv_cla__decode_kernel(
    A_x: jax.Array,
    A_k_cache: jax.Array,
    A_v_cache: jax.Array,
    A_wq: jax.Array,
    A_wo: jax.Array,
    B_x: jax.Array,
    B_c_kv: jax.Array,
    B_w_q: jax.Array,
    B_w_uk: jax.Array,
    B_w_uv: jax.Array,
    B_w_o: jax.Array,
):
    NB, _, DM = A_x.shape
    _, H, S, D = A_k_cache.shape
    DC = B_c_kv.shape[2]
    NH = NB * H
    out = _make_call(NB, H, S, D, DM, DC)(
        A_x.reshape(NB, DM), A_k_cache.reshape(NH * S, D), A_v_cache.reshape(NH * S, D), A_wq, A_wo,
        B_x.reshape(NB, DM), B_c_kv.reshape(NB * S, DC),
        B_w_q.reshape(DM * H, D), B_w_uk.reshape(DC * H, D), B_w_uv.reshape(DC * H, D),
        B_w_o.reshape(H * D, DM),
    )
    return out.reshape(NB, 1, 2 * DM)
```

```python
import jax
import jax.numpy as jnp
import jax.experimental.pallas as pl
import jax.experimental.pallas.tpu as pltpu

_NT = (((1,), (1,)), ((), ()))
_NN = (((1,), (0,)), ((), ()))
_TN = (((0,), (0,)), ((), ()))
_LOG2E = 1.4426950408889634

TILE = 128
CH = 64
DESC_BYTES = 32768


def _dot(a, b, dims):
    return jax.lax.dot_general(a, b, dims, preferred_element_type=jnp.float32)


def _build_kernel(NB, H, S, D, DM, DC, ckv_big_rows):
    NH = NB * H
    NTS = S // TILE
    KH = S // 2
    VQ = S // 4
    CR = DESC_BYTES // (2 * DM)
    scale_log2e = (D ** -0.5) * _LOG2E
    assert NB == 2 and NH <= 128 and D == 128 and DM == DC and NTS % 4 == 0 and NH >= 3
    ckv_half = (NB * S - ckv_big_rows) // 2
    assert ckv_big_rows % CR == 0 and ckv_half % CR == 0 and 2 * ckv_half + ckv_big_rows == NB * S

    def kernel(xa_hbm, k_hbm, v_hbm, wq_hbm, wo_hbm, xb_hbm, ckv_hbm, wqb_hbm, wuk_hbm, wuv_hbm, wob_hbm,
               out_ref,
               xa_v, xb_v, wq_v, wo_v, ckv_v, wqb_v, wuk_v, wuv_v, wob_v,
               kbuf, vbuf, sbuf, qa_s, xbc_s, t_s, ql_s, cl_s,
               sems):
        SEM_XA, SEM_WQ, SEM_XB, SEM_WQB, SEM_WUK = 2, 3, 4, 5, 6
        SEM_CKV_A, SEM_CKV_B, SEM_CKV_C, SEM_WUV, SEM_WOB = 7, 8, 9, 10, 11
        SEM_WO = SEM_CKV_B

        def cp(src, dst, sem):
            return pltpu.make_async_copy(src, dst, sems.at[sem])

        def issue_pairs(n, mk0, mk1, unroll=4):
            assert n % unroll == 0

            def body(i, c):
                for u in range(unroll):
                    mk0(i * unroll + u).start(priority=0)
                    mk1(i * unroll + u).start(priority=1)
                return c
            jax.lax.fori_loop(0, n // unroll, body, 0)

        def rows_chunk(hbm, vmem, sem, nrows, base=0):
            assert base % nrows == 0

            def mk(i):
                r = pl.ds(pl.multiple_of(base + i * nrows, nrows), nrows)
                return cp(hbm.at[r, :], vmem.at[r, :], sem)
            return mk

        def pad_rows(r0, r1):
            n = r0.shape[1]
            rows = jax.lax.broadcasted_iota(jnp.int32, (8, n), 0)
            return jnp.where(rows == 0, jnp.broadcast_to(r0, (8, n)),
                             jnp.where(rows == 1, jnp.broadcast_to(r1, (8, n)), 0.0)).astype(jnp.bfloat16)

        cp(xb_hbm, xb_v, SEM_XB).start()
        cp(xa_hbm, xa_v, SEM_XA).start()
        issue_pairs((DM * H) // TILE,
                    rows_chunk(wqb_hbm, wqb_v, SEM_WQB, TILE), rows_chunk(wuk_hbm, wuk_v, SEM_WUK, TILE))
        ckv_a = cp(ckv_hbm.at[pl.ds(0, ckv_big_rows), :], ckv_v.at[pl.ds(0, ckv_big_rows), :], SEM_CKV_A)
        ckv_a.start(priority=1)

        cp(xb_hbm, xb_v, SEM_XB).wait()
        cp(wqb_hbm, wqb_v, SEM_WQB).wait()
        xbf = xb_v[...].astype(jnp.float32)
        for b in range(NB):
            xbc_s[b] = jnp.broadcast_to(xbf[b:b + 1, :], (128, DM)).T

        def b1_body(m, carry):
            a0, a1 = carry
            w = wqb_v[pl.ds(pl.multiple_of(m * H, H), H), :].astype(jnp.float32)
            return a0 + w * xbc_s[0, pl.ds(m, 1), :], a1 + w * xbc_s[1, pl.ds(m, 1), :]
        zq = jnp.zeros((H, D), jnp.float32)
        qb0, qb1 = jax.lax.fori_loop(0, DM, b1_body, (zq, zq), unroll=8)
        qm = jnp.concatenate([qb0, qb1, jnp.zeros((128 - NH, D), jnp.float32)], axis=0).astype(jnp.bfloat16)

        cp(wuk_hbm, wuk_v, SEM_WUK).wait()
        rows2 = jax.lax.broadcasted_iota(jnp.int32, (CH * H, 128), 0)
        lanes2 = jax.lax.broadcasted_iota(jnp.int32, (CH * H, 128), 1)
        mask2 = (rows2 % H) == (lanes2 % H)

        def b2_chunk(i, c):
            w = wuk_v[pl.ds(pl.multiple_of(i * CH * H, CH * H), CH * H), :]
            o = _dot(w, qm, _NT)
            o = jnp.where(mask2, o, 0.0).reshape(CH, H, 128)
            t_s[pl.ds(pl.multiple_of(i * CH, CH), CH), :] = jnp.sum(o, axis=1)
            return c
        jax.lax.fori_loop(0, DC // CH, b2_chunk, 0)
        ql_s[...] = t_s[...].T

        issue_pairs(ckv_half // CR,
                    rows_chunk(ckv_hbm, ckv_v, SEM_CKV_B, CR, ckv_big_rows),
                    rows_chunk(ckv_hbm, ckv_v, SEM_CKV_C, CR, ckv_big_rows + ckv_half))
        cp(wuv_hbm, wuv_v, SEM_WUV).start(priority=1)
        cp(wob_hbm, wob_v, SEM_WOB).start(priority=1)

        ckv_a.wait()
        r_b = pl.ds(ckv_big_rows, ckv_half)
        r_c = pl.ds(ckv_big_rows + ckv_half, ckv_half)
        cp(ckv_hbm.at[r_b, :], ckv_v.at[r_b, :], SEM_CKV_B).wait()
        cp(ckv_hbm.at[r_c, :], ckv_v.at[r_c, :], SEM_CKV_C).wait()
        for b in range(NB):
            qlb = ql_s[pl.ds(b * H, H), :].astype(jnp.bfloat16)
            c = ckv_v[pl.ds(b * S, S), :]
            s = _dot(qlb, c, _NT)
            m = jnp.max(s, axis=1, keepdims=True)
            p = jnp.exp2((s - m) * scale_log2e)
            l = jnp.sum(p, axis=1, keepdims=True)
            cl = _dot(p.astype(jnp.bfloat16), c, _NN)
            cl_s[pl.ds(b * H, H), :] = cl / l
        cl_s[pl.ds(NH, 128 - NH), :] = jnp.zeros((128 - NH, DC), jnp.float32)

        ncb = wq_hbm.shape[1] // (DESC_BYTES // 16)

        def wq_chunk(i):
            r = pl.ds(pl.multiple_of((i // ncb) * 8, 8), 8)
            c = pl.ds(pl.multiple_of((i % ncb) * (DESC_BYTES // 16), DESC_BYTES // 16), DESC_BYTES // 16)
            return cp(wq_hbm.at[r, c], wq_v.at[r, c], SEM_WQ)
        issue_pairs((DM // 8) * ncb, wq_chunk, rows_chunk(wo_hbm, wo_v, SEM_WO, CR))

        def k_part(slot, part):
            return cp(k_hbm.at[pl.ds(part * KH, KH), :], kbuf.at[slot, pl.ds(part * KH, KH), :], slot * 2 + part)

        def v_part(slot, part):
            return cp(v_hbm.at[pl.ds(part * VQ, VQ), :], vbuf.at[slot, pl.ds(part * VQ, VQ), :],
                      4 + slot * 4 + part)
        for part in range(2):
            k_part(0, part).start(priority=1)
        for part in range(4):
            v_part(0, part).start(priority=1)

        cp(wuv_hbm, wuv_v, SEM_WUV).wait()
        t_s[...] = cl_s[...].T
        rows5 = jax.lax.broadcasted_iota(jnp.int32, (CH, H, 128), 1)
        lanes5 = jax.lax.broadcasted_iota(jnp.int32, (CH, H, 128), 2)
        mask5 = rows5 == (lanes5 % H)

        def b5_chunk(i, acc):
            yt = t_s[pl.ds(pl.multiple_of(i * CH, CH), CH), :]
            zz = jnp.where(mask5, jnp.broadcast_to(yt[:, None, :], (CH, H, 128)), 0.0)
            zz = zz.reshape(CH * H, 128).astype(jnp.bfloat16)
            w = wuv_v[pl.ds(pl.multiple_of(i * CH * H, CH * H), CH * H), :]
            return acc + _dot(zz, w, _TN)
        ctx = jax.lax.fori_loop(0, DC // CH, b5_chunk, jnp.zeros((128, D), jnp.float32))

        cp(wob_hbm, wob_v, SEM_WOB).wait()
        out_b = jnp.zeros((8, DM), jnp.float32)
        for hh in range(H):
            lhs = pad_rows(ctx[hh:hh + 1, :], ctx[H + hh:H + hh + 1, :])
            out_b = out_b + _dot(lhs, wob_v[pl.ds(hh * D, D), :], _NN)
        out_ref[:, pl.ds(DM, DM)] = out_b[0:NB].astype(out_ref.dtype)

        cp(xa_hbm, xa_v, SEM_XA).wait()
        cp(wq_hbm, wq_v, SEM_WQ).wait()
        xaf = xa_v[...].astype(jnp.float32)
        qa = _dot(pad_rows(xaf[0:1], xaf[1:2]), wq_v[...], _NN).astype(jnp.bfloat16).astype(jnp.float32)
        for b in range(NB):
            for hh in range(H):
                qa_s[pl.ds(b * H + hh, 1), :] = qa[b:b + 1, hh * D:(hh + 1) * D]

        def start_k(h, j, prio):
            slot = h % 2
            cp(k_hbm.at[pl.ds(pl.multiple_of(h * S + j * TILE, TILE), TILE), :],
               kbuf.at[slot, pl.ds(j * TILE, TILE), :], slot * 2 + j // (NTS // 2)).start(priority=prio)

        def start_v(h, j, prio):
            slot = h % 2
            cp(v_hbm.at[pl.ds(pl.multiple_of(h * S + j * TILE, TILE), TILE), :],
               vbuf.at[slot, pl.ds(j * TILE, TILE), :], 4 + slot * 4 + j // (NTS // 4)).start(priority=prio)

        def get_q(h):
            return jnp.broadcast_to(qa_s[pl.ds(h, 1), :], (8, D)).astype(jnp.bfloat16)

        rows8 = jax.lax.broadcasted_iota(jnp.int32, (8, D), 0)

        def finish_head(h, acc, l, out_a):
            o = (acc / l).astype(jnp.bfloat16).astype(jnp.float32)
            o = jnp.where(rows8 == h // H, o, 0.0).astype(jnp.bfloat16)
            r = pl.ds(pl.multiple_of((h % H) * D, D), D)
            return out_a + _dot(o, wo_v[r, :], _NN)

        def step(s_, carry):
            m_prev, out_a = carry
            q1 = get_q(s_)
            ks = s_ % 2
            vs = (s_ + 1) % 2
            mrun = jnp.full((8, TILE), -jnp.inf, jnp.float32)
            lrun = jnp.zeros((8, TILE), jnp.float32)
            acc = jnp.zeros((8, D), jnp.float32)
            for j in range(NTS):
                if j % (NTS // 2) == 0:
                    k_part(ks, j // (NTS // 2)).wait()
                if j % (NTS // 4) == 0:
                    v_part(vs, j // (NTS // 4)).wait()
                start_k(s_ + 1, j, 0)
                start_v(s_, j, 1)
                col = pl.ds(j * TILE, TILE)
                p = jnp.exp2((sbuf[vs, :, col] - m_prev) * scale_log2e)
                lrun = lrun + p
                acc = acc + _dot(p.astype(jnp.bfloat16), vbuf[vs, col, :], _NN)
                sc = _dot(q1, kbuf[ks, col, :], _NT)
                sbuf[ks, :, col] = sc
                mrun = jnp.maximum(mrun, sc)
            out_a = finish_head(s_ - 1, acc, jnp.sum(lrun, axis=1, keepdims=True), out_a)
            return jnp.max(mrun, axis=1, keepdims=True), out_a

        def qk_half(h, q1, part):
            k_part(h % 2, part).wait()
            col = pl.ds(part * KH, KH)
            sc = _dot(q1, kbuf[h % 2, col, :], _NT)
            sbuf[h % 2, :, col] = sc
            return jnp.max(sc, axis=1, keepdims=True)

        def pv_rows(h, m, row0, nrows, acc, lsum):
            col = pl.ds(row0, nrows)
            p = jnp.exp2((sbuf[h % 2, :, col] - m) * scale_log2e)
            return (acc + _dot(p.astype(jnp.bfloat16), vbuf[h % 2, col, :], _NN),
                    lsum + jnp.sum(p, axis=1, keepdims=True))

        def split_pairs(start, h, j0, j1):
            for j in range(j0, j1):
                start(h, j, 0)
                start(h, j + NTS // 2, 1)

        cp(wo_hbm, wo_v, SEM_WO).wait()
        q_first = get_q(0)
        split_pairs(start_k, 1, 0, NTS // 4)
        m_a = qk_half(0, q_first, 0)
        split_pairs(start_k, 1, NTS // 4, NTS // 2)
        m_first = jnp.maximum(m_a, qk_half(0, q_first, 1))
        m_prev, out_a = jax.lax.fori_loop(1, NH - 1, step, (m_first, jnp.zeros((8, DM), jnp.float32)))
        hl = NH - 1
        q_last = get_q(hl)
        split_pairs(start_v, hl, 0, NTS // 4)
        m_a = qk_half(hl, q_last, 0)
        split_pairs(start_v, hl, NTS // 4, NTS // 2)
        m_last = jnp.maximum(m_a, qk_half(hl, q_last, 1))
        zacc = jnp.zeros((8, D), jnp.float32)
        zl = jnp.zeros((8, 1), jnp.float32)
        for part in range(4):
            v_part((hl - 1) % 2, part).wait()
        acc, lsum = pv_rows(hl - 1, m_prev, 0, S, zacc, zl)
        out_a = finish_head(hl - 1, acc, lsum, out_a)
        acc, lsum = zacc, zl
        for part in range(4):
            v_part(hl % 2, part).wait()
            acc, lsum = pv_rows(hl, m_last, part * VQ, VQ, acc, lsum)
        out_a = finish_head(hl, acc, lsum, out_a)
        out_ref[:, pl.ds(0, DM)] = out_a[0:NB].astype(out_ref.dtype)

    return kernel


def _make_call(NB, H, S, D, DM, DC, ckv_big_rows=5120, interpret=False):
    NH = NB * H
    bf, f32 = jnp.bfloat16, jnp.float32
    scratch = [
        pltpu.VMEM((NB, DM), bf), pltpu.VMEM((NB, DM), bf),
        pltpu.VMEM((DM, H * D), bf), pltpu.VMEM((H * D, DM), bf),
        pltpu.VMEM((NB * S, DC), bf),
        pltpu.VMEM((DM * H, D), bf), pltpu.VMEM((DC * H, D), bf), pltpu.VMEM((DC * H, D), bf),
        pltpu.VMEM((H * D, DM), bf),
        pltpu.VMEM((2, S, D), bf), pltpu.VMEM((2, S, D), bf),
        pltpu.VMEM((2, 8, S), f32),
        pltpu.VMEM((NH, D), f32),
        pltpu.VMEM((NB, DM, 128), f32),
        pltpu.VMEM((DC, 128), f32), pltpu.VMEM((128, DC), f32), pltpu.VMEM((128, DC), f32),
        pltpu.SemaphoreType.DMA((12,)),
    ]
    return pl.pallas_call(
        _build_kernel(NB, H, S, D, DM, DC, ckv_big_rows),
        out_shape=jax.ShapeDtypeStruct((NB, 2 * DM), bf),
        in_specs=[pl.BlockSpec(memory_space=pl.ANY)] * 11,
        out_specs=pl.BlockSpec(memory_space=pltpu.VMEM),
        scratch_shapes=scratch,
        compiler_params=pltpu.CompilerParams(vmem_limit_bytes=100 * 2**20),
        interpret=interpret,
    )


def _run(A_x, A_k_cache, A_v_cache, A_wq, A_wo, B_x, B_c_kv, B_w_q, B_w_uk, B_w_uv, B_w_o, **kw):
    NB, _, DM = A_x.shape
    _, H, S, D = A_k_cache.shape
    DC = B_c_kv.shape[2]
    NH = NB * H
    out = _make_call(NB, H, S, D, DM, DC, **kw)(
        A_x.reshape(NB, DM), A_k_cache.reshape(NH * S, D), A_v_cache.reshape(NH * S, D), A_wq, A_wo,
        B_x.reshape(NB, DM), B_c_kv.reshape(NB * S, DC),
        B_w_q.reshape(DM * H, D), B_w_uk.reshape(DC * H, D), B_w_uv.reshape(DC * H, D),
        B_w_o.reshape(H * D, DM),
    )
    return out.reshape(NB, 1, 2 * DM)


@jax.jit
def pallas_concat_heads__gqa_block_cached__compressed_kv_cla__decode_kernel(
    A_x: jax.Array,
    A_k_cache: jax.Array,
    A_v_cache: jax.Array,
    A_wq: jax.Array,
    A_wo: jax.Array,
    B_x: jax.Array,
    B_c_kv: jax.Array,
    B_w_q: jax.Array,
    B_w_uk: jax.Array,
    B_w_uv: jax.Array,
    B_w_o: jax.Array,
):
    return _run(A_x, A_k_cache, A_v_cache, A_wq, A_wo, B_x, B_c_kv, B_w_q, B_w_uk, B_w_uv, B_w_o)
```

```python
import jax
import jax.numpy as jnp
import jax.experimental.pallas as pl
import jax.experimental.pallas.tpu as pltpu

_NT = (((1,), (1,)), ((), ()))
_NN = (((1,), (0,)), ((), ()))
_TN = (((0,), (0,)), ((), ()))
_LOG2E = 1.4426950408889634

TILE = 128
CH = 8
DESC_BYTES = 32768
N_SEMS = 12


def _dot(a, b, dims):
    return jax.lax.dot_general(a, b, dims, preferred_element_type=jnp.float32)


def _build_kernel(NB, H, S, D, DM, DC):
    NH = NB * H
    NTS = S // TILE
    KH = S // 2
    VQ = S // 4
    CR = DESC_BYTES // (2 * DM)
    CQ = S // 4
    WQC = DESC_BYTES // 16
    B1_TRIPS = CQ // CR
    scale_log2e = (D ** -0.5) * _LOG2E
    assert NB == 2 and NH <= 128 and D == 128 and DM == DC and NTS % 8 == 0 and NH >= 3
    assert DM % B1_TRIPS == 0 and (H * D) % WQC == 0 and DC % CH == 0
    WUV0, KB0 = DC * H, 2 * DC * H
    VB0 = KB0 + 2 * S
    WOB0 = NB * S
    WOA0 = WOB0 + H * D

    def kernel(xa_hbm, k_hbm, v_hbm, wq_hbm, wo_hbm, xb_hbm, ckv_hbm, wqb_hbm, wuk_hbm, wuv_hbm, wob_hbm,
               out_ref,
               xa_v, xb_v, wq_v, wqb_v, wide, pool,
               sa_s, sb_s, qa_s, xbc_s, t_s, ql_s, cl_s,
               sems):
        SEM_XA, SEM_WQ = 2, 3
        SEM_XB, SEM_WQB, SEM_WUK = 4, 5, 6
        SEM_C0 = (7, 10, 8, 11)
        SEM_WUV = (5, 9)
        SEM_C1 = (4, 6)
        SEM_WOB, SEM_WOA = 7, 8

        def cp(src, dst, sem):
            return pltpu.make_async_copy(src, dst, sems.at[sem])

        def rows_of(hbm, vmem, nrows, sem, src0=0, dst0=0):
            assert src0 % nrows == 0 and dst0 % nrows == 0

            def mk(i):
                return cp(hbm.at[pl.ds(pl.multiple_of(src0 + i * nrows, nrows), nrows), :],
                          vmem.at[pl.ds(pl.multiple_of(dst0 + i * nrows, nrows), nrows), :], sem)
            return mk

        def wait_rows(vmem, row0, nrows, sem):
            view = vmem.at[pl.ds(row0, nrows), :]
            cp(view, view, sem).wait()

        def start_pair(d0, d1):
            d0.start(priority=0)
            d1.start(priority=1)

        def issue_pairs(n, mk0, mk1, unroll=4):
            assert n % unroll == 0

            def body(i, c):
                for u in range(unroll):
                    start_pair(mk0(i * unroll + u), mk1(i * unroll + u))
                return c
            jax.lax.fori_loop(0, n // unroll, body, 0)

        def spread(n_pairs, n_slots, mk0, mk1):
            def enqueue(slot):
                for i in range(slot * n_pairs // n_slots, (slot + 1) * n_pairs // n_slots):
                    start_pair(mk0(i), mk1(i))
            return enqueue

        def pad_rows(r0, r1):
            n = r0.shape[1]
            rows = jax.lax.broadcasted_iota(jnp.int32, (8, n), 0)
            return jnp.where(rows == 0, jnp.broadcast_to(r0, (8, n)),
                             jnp.where(rows == 1, jnp.broadcast_to(r1, (8, n)), 0.0)).astype(jnp.bfloat16)

        cp(xb_hbm, xb_v, SEM_XB).start()
        cp(xa_hbm, xa_v, SEM_XA).start()
        issue_pairs(DM * H // TILE, rows_of(wqb_hbm, wqb_v, TILE, SEM_WQB), rows_of(wuk_hbm, pool, TILE, SEM_WUK))

        cp(xb_hbm, xb_v, SEM_XB).wait()
        wait_rows(wqb_v, 0, DM * H, SEM_WQB)
        xbf = xb_v[...].astype(jnp.float32)
        for b in range(NB):
            xbc_s[b] = jnp.broadcast_to(xbf[b:b + 1, :], (128, DM)).T
        ckv0 = [rows_of(ckv_hbm, wide, CR, SEM_C0[q], q * CQ, q * CQ) for q in range(4)]

        def b1_body(i, carry):
            a0, a1 = carry
            start_pair(ckv0[0](i), ckv0[2](i))
            for u in range(DM // B1_TRIPS):
                m = i * (DM // B1_TRIPS) + u
                w = wqb_v[pl.ds(pl.multiple_of(m * H, H), H), :].astype(jnp.float32)
                a0 = a0 + w * xbc_s[0, pl.ds(m, 1), :]
                a1 = a1 + w * xbc_s[1, pl.ds(m, 1), :]
            return a0, a1
        zq = jnp.zeros((H, D), jnp.float32)
        qb0, qb1 = jax.lax.fori_loop(0, B1_TRIPS, b1_body, (zq, zq))
        qt = jnp.concatenate([qb0, qb1, jnp.zeros((128 - NH, D), jnp.float32)], axis=0).T.astype(jnp.bfloat16)

        wait_rows(pool, 0, DC * H, SEM_WUK)
        rows2 = jax.lax.broadcasted_iota(jnp.int32, (CH * H, 128), 0)
        lanes2 = jax.lax.broadcasted_iota(jnp.int32, (CH * H, 128), 1)
        mask2 = (rows2 % H) == (lanes2 % H)
        enqueue = spread(DC * H // TILE // 2, DC // CH,
                         rows_of(wuv_hbm, pool, TILE, SEM_WUV[0], 0, WUV0),
                         rows_of(wuv_hbm, pool, TILE, SEM_WUV[1], DC * H // 2, WUV0 + DC * H // 2))
        for i in range(DC // CH):
            enqueue(i)
            o = _dot(pool[pl.ds(i * CH * H, CH * H), :], qt, _NN)
            o = jnp.where(mask2, o, 0.0).reshape(CH, H, 128)
            t_s[pl.ds(i * CH, CH), :] = jnp.sum(o, axis=1)
        ql_s[...] = t_s[...].T

        issue_pairs(B1_TRIPS, ckv0[1], ckv0[3])

        def latent_attention(b, enqueue, waits):
            qlb = ql_s[pl.ds(b * H, H), :].astype(jnp.bfloat16)
            mrun = jnp.full((H, TILE), -jnp.inf, jnp.float32)
            for j in range(NTS):
                enqueue(j)
                if j in waits:
                    wait_rows(wide, *waits[j])
                sc = _dot(qlb, wide[pl.ds(b * S + j * TILE, TILE), :], _NT)
                sb_s[:, pl.ds(j * TILE, TILE)] = sc
                mrun = jnp.maximum(mrun, sc)
            m = jnp.max(mrun, axis=1, keepdims=True)
            lrun = jnp.zeros((H, TILE), jnp.float32)
            cl = jnp.zeros((H, DC), jnp.float32)
            for j in range(NTS):
                enqueue(NTS + j)
                p = jnp.exp2((sb_s[:, pl.ds(j * TILE, TILE)] - m) * scale_log2e)
                lrun = lrun + p
                cl = cl + _dot(p.astype(jnp.bfloat16), wide[pl.ds(b * S + j * TILE, TILE), :], _NN)
            cl_s[pl.ds(b * H, H), :] = cl / jnp.sum(lrun, axis=1, keepdims=True)

        latent_attention(
            0,
            spread(S // 2 // CR, 2 * NTS, rows_of(ckv_hbm, wide, CR, SEM_C1[0], S, S),
                   rows_of(ckv_hbm, wide, CR, SEM_C1[1], S + S // 2, S + S // 2)),
            {q * NTS // 4: (q * CQ, CQ, SEM_C0[q]) for q in range(4)})
        latent_attention(
            1,
            spread(H * D // CR, 2 * NTS, rows_of(wob_hbm, wide, CR, SEM_WOB, 0, WOB0),
                   rows_of(wo_hbm, wide, CR, SEM_WOA, 0, WOA0)),
            {0: (S, S // 2, SEM_C1[0]), NTS // 2: (S + S // 2, S // 2, SEM_C1[1])})
        cl_s[pl.ds(NH, 128 - NH), :] = jnp.zeros((128 - NH, DC), jnp.float32)

        ncb = H * D // WQC
        n_wq = (DM // 8) * ncb

        def wq_strip(i0):
            def mk(i):
                r = pl.ds(pl.multiple_of(((i0 + i) // ncb) * 8, 8), 8)
                c = pl.ds(pl.multiple_of(((i0 + i) % ncb) * WQC, WQC), WQC)
                return cp(wq_hbm.at[r, c], wq_v.at[r, c], SEM_WQ)
            return mk
        issue_pairs(n_wq // 2, wq_strip(0), wq_strip(n_wq // 2))

        def k_chunk(h, j):
            slot = h % 2
            return cp(k_hbm.at[pl.ds(pl.multiple_of(h * S + j * TILE, TILE), TILE), :],
                      pool.at[pl.ds(pl.multiple_of(KB0 + slot * S + j * TILE, TILE), TILE), :],
                      slot * 2 + j // (NTS // 2))

        def v_chunk(h, j):
            slot = h % 2
            return cp(v_hbm.at[pl.ds(pl.multiple_of(h * S + j * TILE, TILE), TILE), :],
                      pool.at[pl.ds(pl.multiple_of(VB0 + slot * S + j * TILE, TILE), TILE), :],
                      4 + slot * 4 + j // (NTS // 4))

        wait_rows(wide, WOB0, H * D, SEM_WOB)
        wait_rows(pool, WUV0, DC * H // 2, SEM_WUV[0])
        wait_rows(pool, WUV0 + DC * H // 2, DC * H // 2, SEM_WUV[1])
        t_s[...] = cl_s[...].T
        rows5 = jax.lax.broadcasted_iota(jnp.int32, (CH, H, 128), 1)
        lanes5 = jax.lax.broadcasted_iota(jnp.int32, (CH, H, 128), 2)
        mask5 = rows5 == (lanes5 % H)
        enqueue = spread(NTS, DC // CH, lambda j: k_chunk(0, j), lambda j: v_chunk(0, j))
        ctx = jnp.zeros((NH, D), jnp.float32)
        for i in range(DC // CH):
            enqueue(i)
            yt = t_s[pl.ds(i * CH, CH), :]
            zz = jnp.where(mask5, jnp.broadcast_to(yt[:, None, :], (CH, H, 128)), 0.0)
            zz = zz.reshape(CH * H, 128).astype(jnp.bfloat16)[:, :NH]
            ctx = ctx + _dot(zz, pool[pl.ds(WUV0 + i * CH * H, CH * H), :], _TN)

        def k_wait(slot, part):
            wait_rows(pool, pl.multiple_of(KB0 + slot * S + part * KH, TILE), KH, slot * 2 + part)

        def v_wait(slot, part):
            wait_rows(pool, pl.multiple_of(VB0 + slot * S + part * VQ, TILE), VQ, 4 + slot * 4 + part)

        def k_rows(slot, row0, nrows):
            return pool[pl.ds(pl.multiple_of(KB0 + slot * S + row0, TILE), nrows), :]

        def v_rows(slot, row0, nrows):
            return pool[pl.ds(pl.multiple_of(VB0 + slot * S + row0, TILE), nrows), :]

        def get_q(h):
            return jnp.broadcast_to(qa_s[pl.ds(h, 1), :], (8, D)).astype(jnp.bfloat16)

        rows8 = jax.lax.broadcasted_iota(jnp.int32, (8, D), 0)

        def finish_head(h, acc, l, out_a):
            o = (acc / l).astype(jnp.bfloat16).astype(jnp.float32)
            o = jnp.where(rows8 == h // H, o, 0.0).astype(jnp.bfloat16)
            r = pl.ds(pl.multiple_of(WOA0 + (h % H) * D, D), D)
            return out_a + _dot(o, wide[r, :], _NN)

        def step(s_, carry):
            m_prev, out_a = carry
            q1 = get_q(s_)
            ks = s_ % 2
            vs = (s_ + 1) % 2
            mrun = jnp.full((8, TILE), -jnp.inf, jnp.float32)
            lrun = jnp.zeros((8, TILE), jnp.float32)
            acc = jnp.zeros((8, D), jnp.float32)
            for j in range(NTS):
                if j % (NTS // 2) == 0:
                    k_wait(ks, j // (NTS // 2))
                if j % (NTS // 4) == 0:
                    v_wait(vs, j // (NTS // 4))
                start_pair(k_chunk(s_ + 1, j), v_chunk(s_, j))
                col = pl.ds(j * TILE, TILE)
                p = jnp.exp2((sa_s[vs, :, col] - m_prev) * scale_log2e)
                lrun = lrun + p
                acc = acc + _dot(p.astype(jnp.bfloat16), v_rows(vs, j * TILE, TILE), _NN)
                sc = _dot(q1, k_rows(ks, j * TILE, TILE), _NT)
                sa_s[ks, :, col] = sc
                mrun = jnp.maximum(mrun, sc)
            out_a = finish_head(s_ - 1, acc, jnp.sum(lrun, axis=1, keepdims=True), out_a)
            return jnp.max(mrun, axis=1, keepdims=True), out_a

        def qk_half(h, q1, part):
            k_wait(h % 2, part)
            sc = _dot(q1, k_rows(h % 2, part * KH, KH), _NT)
            sa_s[h % 2, :, pl.ds(part * KH, KH)] = sc
            return jnp.max(sc, axis=1, keepdims=True)

        def pv_rows(h, m, row0, nrows, acc, lsum):
            p = jnp.exp2((sa_s[h % 2, :, pl.ds(row0, nrows)] - m) * scale_log2e)
            return (acc + _dot(p.astype(jnp.bfloat16), v_rows(h % 2, row0, nrows), _NN),
                    lsum + jnp.sum(p, axis=1, keepdims=True))

        g = NTS // 8

        def split_pairs(chunk, h, part):
            for j in range(part * g, (part + 1) * g):
                start_pair(chunk(h, j), chunk(h, j + NTS // 2))

        zacc = jnp.zeros((8, D), jnp.float32)
        zl = jnp.zeros((8, 1), jnp.float32)

        cp(xa_hbm, xa_v, SEM_XA).wait()
        wait_rows(wq_v, 0, DM, SEM_WQ)
        split_pairs(k_chunk, 1, 0)
        out_b = jnp.zeros((8, DM), jnp.float32)
        for hh in range(H):
            lhs = pad_rows(ctx[hh:hh + 1, :], ctx[H + hh:H + hh + 1, :])
            out_b = out_b + _dot(lhs, wide[pl.ds(WOB0 + hh * D, D), :], _NN)
        out_ref[:, pl.ds(DM, DM)] = out_b[0:NB].astype(out_ref.dtype)
        split_pairs(k_chunk, 1, 1)
        xaf = xa_v[...].astype(jnp.float32)
        qa = _dot(pad_rows(xaf[0:1], xaf[1:2]), wq_v[...], _NN).astype(jnp.bfloat16).astype(jnp.float32)
        for b in range(NB):
            for hh in range(H):
                qa_s[pl.ds(b * H + hh, 1), :] = qa[b:b + 1, hh * D:(hh + 1) * D]
        q_first = get_q(0)
        split_pairs(k_chunk, 1, 2)
        m_a = qk_half(0, q_first, 0)
        split_pairs(k_chunk, 1, 3)
        m_first = jnp.maximum(m_a, qk_half(0, q_first, 1))
        wait_rows(wide, WOA0, H * D, SEM_WOA)

        m_prev, out_a = jax.lax.fori_loop(1, NH - 1, step, (m_first, jnp.zeros((8, DM), jnp.float32)))

        hl = NH - 1
        q_last = get_q(hl)
        split_pairs(v_chunk, hl, 0)
        m_a = qk_half(hl, q_last, 0)
        split_pairs(v_chunk, hl, 1)
        m_last = jnp.maximum(m_a, qk_half(hl, q_last, 1))
        split_pairs(v_chunk, hl, 2)
        for part in range(2):
            v_wait((hl - 1) % 2, part)
        acc, lsum = pv_rows(hl - 1, m_prev, 0, S // 2, zacc, zl)
        split_pairs(v_chunk, hl, 3)
        for part in range(2, 4):
            v_wait((hl - 1) % 2, part)
        acc, lsum = pv_rows(hl - 1, m_prev, S // 2, S // 2, acc, lsum)
        out_a = finish_head(hl - 1, acc, lsum, out_a)
        acc, lsum = zacc, zl
        for part in range(4):
            v_wait(hl % 2, part)
            acc, lsum = pv_rows(hl, m_last, part * VQ, VQ, acc, lsum)
        out_a = finish_head(hl, acc, lsum, out_a)
        out_ref[:, pl.ds(0, DM)] = out_a[0:NB].astype(out_ref.dtype)

    return kernel


def _make_call(NB, H, S, D, DM, DC, interpret=False):
    NH = NB * H
    bf, f32 = jnp.bfloat16, jnp.float32
    scratch = [
        pltpu.VMEM((NB, DM), bf), pltpu.VMEM((NB, DM), bf),
        pltpu.VMEM((DM, H * D), bf),
        pltpu.VMEM((DM * H, D), bf),
        pltpu.VMEM((NB * S + 2 * H * D, DM), bf),
        pltpu.VMEM((2 * DC * H + 4 * S, D), bf),
        pltpu.VMEM((2, 8, S), f32),
        pltpu.VMEM((H, S), f32),
        pltpu.VMEM((NH, D), f32),
        pltpu.VMEM((NB, DM, 128), f32),
        pltpu.VMEM((DC, 128), f32),
        pltpu.VMEM((128, DC), f32), pltpu.VMEM((128, DC), f32),
        pltpu.SemaphoreType.DMA((N_SEMS,)),
    ]
    return pl.pallas_call(
        _build_kernel(NB, H, S, D, DM, DC),
        out_shape=jax.ShapeDtypeStruct((NB, 2 * DM), bf),
        in_specs=[pl.BlockSpec(memory_space=pl.ANY)] * 11,
        out_specs=pl.BlockSpec(memory_space=pltpu.VMEM),
        scratch_shapes=scratch,
        compiler_params=pltpu.CompilerParams(vmem_limit_bytes=100 * 2**20),
        interpret=interpret,
    )


def _run(A_x, A_k_cache, A_v_cache, A_wq, A_wo, B_x, B_c_kv, B_w_q, B_w_uk, B_w_uv, B_w_o, **kw):
    NB, _, DM = A_x.shape
    _, H, S, D = A_k_cache.shape
    DC = B_c_kv.shape[2]
    NH = NB * H
    out = _make_call(NB, H, S, D, DM, DC, **kw)(
        A_x.reshape(NB, DM), A_k_cache.reshape(NH * S, D), A_v_cache.reshape(NH * S, D), A_wq, A_wo,
        B_x.reshape(NB, DM), B_c_kv.reshape(NB * S, DC),
        B_w_q.reshape(DM * H, D), B_w_uk.reshape(DC * H, D), B_w_uv.reshape(DC * H, D),
        B_w_o.reshape(H * D, DM),
    )
    return out.reshape(NB, 1, 2 * DM)


@jax.jit
def pallas_concat_heads__gqa_block_cached__compressed_kv_cla__decode_kernel(
    A_x: jax.Array,
    A_k_cache: jax.Array,
    A_v_cache: jax.Array,
    A_wq: jax.Array,
    A_wo: jax.Array,
    B_x: jax.Array,
    B_c_kv: jax.Array,
    B_w_q: jax.Array,
    B_w_uk: jax.Array,
    B_w_uv: jax.Array,
    B_w_o: jax.Array,
):
    return _run(A_x, A_k_cache, A_v_cache, A_wq, A_wo, B_x, B_c_kv, B_w_q, B_w_uk, B_w_uv, B_w_o)
```

```python
import jax
import jax.numpy as jnp
import jax.experimental.pallas as pl
import jax.experimental.pallas.tpu as pltpu

_NT = (((1,), (1,)), ((), ()))
_NN = (((1,), (0,)), ((), ()))
_TN = (((0,), (0,)), ((), ()))
_LOG2E = 1.4426950408889634

TILE = 128
CH = 8
DESC_BYTES = 32768
N_SEMS = 12


def _dot(a, b, dims):
    return jax.lax.dot_general(a, b, dims, preferred_element_type=jnp.float32)


def _hop_order(i, n, fast_bits):
    nbits = n.bit_length() - 1
    assert n == 1 << nbits
    order = [b for b in fast_bits if b < nbits] + [b for b in range(nbits) if b not in fast_bits]
    out = 0
    for k, b in enumerate(order):
        out = out | (((i >> k) & 1) << b)
    return out


def _build_kernel(NB, H, S, D, DM, DC):
    NH = NB * H
    NTS = S // TILE
    KH = S // 2
    VQ = S // 4
    CR = DESC_BYTES // (2 * DM)
    CQ = S // 4
    WQC = DESC_BYTES // 16
    B1_TRIPS = CQ // CR
    key_order = [_hop_order(j, NTS, (4, 5, 2, 3)) for j in range(NTS)]
    scale_log2e = (D ** -0.5) * _LOG2E
    assert NB == 2 and NH <= 128 and D == 128 and DM == DC and NTS % 8 == 0 and NH >= 3
    assert DM % B1_TRIPS == 0 and (H * D) % WQC == 0 and DC % CH == 0
    WUV0, KB0 = DC * H, 2 * DC * H
    VB0 = KB0 + 2 * S
    WOB0 = NB * S
    WOA0 = WOB0 + H * D

    def kernel(xa_hbm, k_hbm, v_hbm, wq_hbm, wo_hbm, xb_hbm, ckv_hbm, wqb_hbm, wuk_hbm, wuv_hbm, wob_hbm,
               out_ref,
               xa_v, xb_v, wq_v, wqb_v, wide, pool,
               sa_s, sb_s, qa_s, xbc_s, t_s, ql_s, cl_s,
               sems):
        SEM_XA, SEM_WQ = 2, 3
        SEM_XB, SEM_WQB, SEM_WUK = 4, 5, 6
        SEM_C0 = (7, 10, 8, 11)
        SEM_WUV = (5, 9)
        SEM_C1 = (4, 6)
        SEM_WOB, SEM_WOA = 7, 8

        def cp(src, dst, sem):
            return pltpu.make_async_copy(src, dst, sems.at[sem])

        def rows_of(hbm, vmem, nrows, n, sem, src0=0, dst0=0):
            assert src0 % nrows == 0 and dst0 % nrows == 0

            def mk(i):
                i = _hop_order(i, n, (6, 5, 4))
                return cp(hbm.at[pl.ds(pl.multiple_of(src0 + i * nrows, nrows), nrows), :],
                          vmem.at[pl.ds(pl.multiple_of(dst0 + i * nrows, nrows), nrows), :], sem)
            return mk

        def wait_rows(vmem, row0, nrows, sem):
            view = vmem.at[pl.ds(row0, nrows), :]
            cp(view, view, sem).wait()

        def start_pair(d0, d1):
            d0.start(priority=0)
            d1.start(priority=1)

        def issue_pairs(n, mk0, mk1, unroll=4):
            assert n % unroll == 0

            def body(i, c):
                for u in range(unroll):
                    start_pair(mk0(i * unroll + u), mk1(i * unroll + u))
                return c
            jax.lax.fori_loop(0, n // unroll, body, 0)

        def spread(n_pairs, n_slots, mk0, mk1):
            def enqueue(slot):
                for i in range(slot * n_pairs // n_slots, (slot + 1) * n_pairs // n_slots):
                    start_pair(mk0(i), mk1(i))
            return enqueue

        def pad_rows(r0, r1):
            n = r0.shape[1]
            rows = jax.lax.broadcasted_iota(jnp.int32, (8, n), 0)
            return jnp.where(rows == 0, jnp.broadcast_to(r0, (8, n)),
                             jnp.where(rows == 1, jnp.broadcast_to(r1, (8, n)), 0.0)).astype(jnp.bfloat16)

        cp(xb_hbm, xb_v, SEM_XB).start()
        cp(xa_hbm, xa_v, SEM_XA).start()
        n_w = DM * H // TILE
        issue_pairs(n_w, rows_of(wqb_hbm, wqb_v, TILE, n_w, SEM_WQB), rows_of(wuk_hbm, pool, TILE, n_w, SEM_WUK))

        cp(xb_hbm, xb_v, SEM_XB).wait()
        wait_rows(wqb_v, 0, DM * H, SEM_WQB)
        xbf = xb_v[...].astype(jnp.float32)
        for b in range(NB):
            xbc_s[b] = jnp.broadcast_to(xbf[b:b + 1, :], (128, DM)).T
        ckv0 = [rows_of(ckv_hbm, wide, CR, B1_TRIPS, SEM_C0[q], q * CQ, q * CQ) for q in range(4)]

        def b1_body(i, carry):
            a0, a1 = carry
            start_pair(ckv0[0](i), ckv0[2](i))
            for u in range(DM // B1_TRIPS):
                m = i * (DM // B1_TRIPS) + u
                w = wqb_v[pl.ds(pl.multiple_of(m * H, H), H), :].astype(jnp.float32)
                a0 = a0 + w * xbc_s[0, pl.ds(m, 1), :]
                a1 = a1 + w * xbc_s[1, pl.ds(m, 1), :]
            return a0, a1
        zq = jnp.zeros((H, D), jnp.float32)
        qb0, qb1 = jax.lax.fori_loop(0, B1_TRIPS, b1_body, (zq, zq))
        qt = jnp.concatenate([qb0, qb1, jnp.zeros((128 - NH, D), jnp.float32)], axis=0).T.astype(jnp.bfloat16)

        wait_rows(pool, 0, DC * H, SEM_WUK)
        rows2 = jax.lax.broadcasted_iota(jnp.int32, (CH * H, 128), 0)
        lanes2 = jax.lax.broadcasted_iota(jnp.int32, (CH * H, 128), 1)
        mask2 = (rows2 % H) == (lanes2 % H)
        n_uv = DC * H // TILE // 2
        enqueue = spread(n_uv, DC // CH,
                         rows_of(wuv_hbm, pool, TILE, n_uv, SEM_WUV[0], 0, WUV0),
                         rows_of(wuv_hbm, pool, TILE, n_uv, SEM_WUV[1], DC * H // 2, WUV0 + DC * H // 2))
        for i in range(DC // CH):
            enqueue(i)
            o = _dot(pool[pl.ds(i * CH * H, CH * H), :], qt, _NN)
            o = jnp.where(mask2, o, 0.0).reshape(CH, H, 128)
            t_s[pl.ds(i * CH, CH), :] = jnp.sum(o, axis=1)
        ql_s[...] = t_s[...].T

        issue_pairs(B1_TRIPS, ckv0[1], ckv0[3])

        def latent_attention(b, enqueue, waits):
            qlb = ql_s[pl.ds(b * H, H), :].astype(jnp.bfloat16)
            mrun = jnp.full((H, TILE), -jnp.inf, jnp.float32)
            for j in range(NTS):
                enqueue(j)
                if j in waits:
                    wait_rows(wide, *waits[j])
                sc = _dot(qlb, wide[pl.ds(b * S + j * TILE, TILE), :], _NT)
                sb_s[:, pl.ds(j * TILE, TILE)] = sc
                mrun = jnp.maximum(mrun, sc)
            m = jnp.max(mrun, axis=1, keepdims=True)
            lrun = jnp.zeros((H, TILE), jnp.float32)
            cl = jnp.zeros((H, DC), jnp.float32)
            for j in range(NTS):
                enqueue(NTS + j)
                p = jnp.exp2((sb_s[:, pl.ds(j * TILE, TILE)] - m) * scale_log2e)
                lrun = lrun + p
                cl = cl + _dot(p.astype(jnp.bfloat16), wide[pl.ds(b * S + j * TILE, TILE), :], _NN)
            cl_s[pl.ds(b * H, H), :] = cl / jnp.sum(lrun, axis=1, keepdims=True)

        n_c1, n_wo = S // 2 // CR, H * D // CR
        latent_attention(
            0,
            spread(n_c1, 2 * NTS, rows_of(ckv_hbm, wide, CR, n_c1, SEM_C1[0], S, S),
                   rows_of(ckv_hbm, wide, CR, n_c1, SEM_C1[1], S + S // 2, S + S // 2)),
            {q * NTS // 4: (q * CQ, CQ, SEM_C0[q]) for q in range(4)})
        latent_attention(
            1,
            spread(n_wo, 2 * NTS, rows_of(wob_hbm, wide, CR, n_wo, SEM_WOB, 0, WOB0),
                   rows_of(wo_hbm, wide, CR, n_wo, SEM_WOA, 0, WOA0)),
            {0: (S, S // 2, SEM_C1[0]), NTS // 2: (S + S // 2, S // 2, SEM_C1[1])})
        cl_s[pl.ds(NH, 128 - NH), :] = jnp.zeros((128 - NH, DC), jnp.float32)

        ncb = H * D // WQC
        n_wq = (DM // 8) * ncb

        def wq_strip(i0):
            def mk(i):
                i = _hop_order(i, n_wq // 2, (6, 5, 4))
                r = pl.ds(pl.multiple_of(((i0 + i) // ncb) * 8, 8), 8)
                c = pl.ds(pl.multiple_of(((i0 + i) % ncb) * WQC, WQC), WQC)
                return cp(wq_hbm.at[r, c], wq_v.at[r, c], SEM_WQ)
            return mk
        issue_pairs(n_wq // 2, wq_strip(0), wq_strip(n_wq // 2))

        def k_chunk(h, j):
            slot = h % 2
            return cp(k_hbm.at[pl.ds(pl.multiple_of(h * S + key_order[j] * TILE, TILE), TILE), :],
                      pool.at[pl.ds(pl.multiple_of(KB0 + slot * S + j * TILE, TILE), TILE), :],
                      slot * 2 + j // (NTS // 2))

        def v_chunk(h, j):
            slot = h % 2
            return cp(v_hbm.at[pl.ds(pl.multiple_of(h * S + key_order[j] * TILE, TILE), TILE), :],
                      pool.at[pl.ds(pl.multiple_of(VB0 + slot * S + j * TILE, TILE), TILE), :],
                      4 + slot * 4 + j // (NTS // 4))

        wait_rows(wide, WOB0, H * D, SEM_WOB)
        wait_rows(pool, WUV0, DC * H // 2, SEM_WUV[0])
        wait_rows(pool, WUV0 + DC * H // 2, DC * H // 2, SEM_WUV[1])
        t_s[...] = cl_s[...].T
        rows5 = jax.lax.broadcasted_iota(jnp.int32, (CH, H, 128), 1)
        lanes5 = jax.lax.broadcasted_iota(jnp.int32, (CH, H, 128), 2)
        mask5 = rows5 == (lanes5 % H)
        enqueue = spread(NTS, DC // CH, lambda j: k_chunk(0, j), lambda j: v_chunk(0, j))
        ctx = jnp.zeros((NH, D), jnp.float32)
        for i in range(DC // CH):
            enqueue(i)
            yt = t_s[pl.ds(i * CH, CH), :]
            zz = jnp.where(mask5, jnp.broadcast_to(yt[:, None, :], (CH, H, 128)), 0.0)
            zz = zz.reshape(CH * H, 128).astype(jnp.bfloat16)[:, :NH]
            ctx = ctx + _dot(zz, pool[pl.ds(WUV0 + i * CH * H, CH * H), :], _TN)

        def k_wait(slot, part):
            wait_rows(pool, pl.multiple_of(KB0 + slot * S + part * KH, TILE), KH, slot * 2 + part)

        def v_wait(slot, part):
            wait_rows(pool, pl.multiple_of(VB0 + slot * S + part * VQ, TILE), VQ, 4 + slot * 4 + part)

        def k_rows(slot, row0, nrows):
            return pool[pl.ds(pl.multiple_of(KB0 + slot * S + row0, TILE), nrows), :]

        def v_rows(slot, row0, nrows):
            return pool[pl.ds(pl.multiple_of(VB0 + slot * S + row0, TILE), nrows), :]

        def get_q(h):
            return jnp.broadcast_to(qa_s[pl.ds(h, 1), :], (8, D)).astype(jnp.bfloat16)

        rows8 = jax.lax.broadcasted_iota(jnp.int32, (8, D), 0)

        def finish_head(h, acc, l, out_a):
            o = (acc / l).astype(jnp.bfloat16).astype(jnp.float32)
            o = jnp.where(rows8 == h // H, o, 0.0).astype(jnp.bfloat16)
            r = pl.ds(pl.multiple_of(WOA0 + (h % H) * D, D), D)
            return out_a + _dot(o, wide[r, :], _NN)

        def step(s_, carry):
            m_prev, out_a = carry
            q1 = get_q(s_)
            ks = s_ % 2
            vs = (s_ + 1) % 2
            mrun = jnp.full((8, TILE), -jnp.inf, jnp.float32)
            lrun = jnp.zeros((8, TILE), jnp.float32)
            acc = jnp.zeros((8, D), jnp.float32)
            for j in range(NTS):
                if j % (NTS // 2) == 0:
                    k_wait(ks, j // (NTS // 2))
                if j % (NTS // 4) == 0:
                    v_wait(vs, j // (NTS // 4))
                start_pair(k_chunk(s_ + 1, j), v_chunk(s_, j))
                col = pl.ds(j * TILE, TILE)
                p = jnp.exp2((sa_s[vs, :, col] - m_prev) * scale_log2e)
                lrun = lrun + p
                acc = acc + _dot(p.astype(jnp.bfloat16), v_rows(vs, j * TILE, TILE), _NN)
                sc = _dot(q1, k_rows(ks, j * TILE, TILE), _NT)
                sa_s[ks, :, col] = sc
                mrun = jnp.maximum(mrun, sc)
            out_a = finish_head(s_ - 1, acc, jnp.sum(lrun, axis=1, keepdims=True), out_a)
            return jnp.max(mrun, axis=1, keepdims=True), out_a

        def qk_half(h, q1, part):
            k_wait(h % 2, part)
            sc = _dot(q1, k_rows(h % 2, part * KH, KH), _NT)
            sa_s[h % 2, :, pl.ds(part * KH, KH)] = sc
            return jnp.max(sc, axis=1, keepdims=True)

        def pv_rows(h, m, row0, nrows, acc, lsum):
            p = jnp.exp2((sa_s[h % 2, :, pl.ds(row0, nrows)] - m) * scale_log2e)
            return (acc + _dot(p.astype(jnp.bfloat16), v_rows(h % 2, row0, nrows), _NN),
                    lsum + jnp.sum(p, axis=1, keepdims=True))

        g = NTS // 8

        def split_pairs(chunk, h, part):
            for j in range(part * g, (part + 1) * g):
                start_pair(chunk(h, j), chunk(h, j + NTS // 2))

        zacc = jnp.zeros((8, D), jnp.float32)
        zl = jnp.zeros((8, 1), jnp.float32)

        cp(xa_hbm, xa_v, SEM_XA).wait()
        wait_rows(wq_v, 0, DM, SEM_WQ)
        split_pairs(k_chunk, 1, 0)
        out_b = jnp.zeros((8, DM), jnp.float32)
        for hh in range(H):
            lhs = pad_rows(ctx[hh:hh + 1, :], ctx[H + hh:H + hh + 1, :])
            out_b = out_b + _dot(lhs, wide[pl.ds(WOB0 + hh * D, D), :], _NN)
        out_ref[:, pl.ds(DM, DM)] = out_b[0:NB].astype(out_ref.dtype)
        split_pairs(k_chunk, 1, 1)
        xaf = xa_v[...].astype(jnp.float32)
        qa = _dot(pad_rows(xaf[0:1], xaf[1:2]), wq_v[...], _NN).astype(jnp.bfloat16).astype(jnp.float32)
        for b in range(NB):
            for hh in range(H):
                qa_s[pl.ds(b * H + hh, 1), :] = qa[b:b + 1, hh * D:(hh + 1) * D]
        q_first = get_q(0)
        split_pairs(k_chunk, 1, 2)
        m_a = qk_half(0, q_first, 0)
        split_pairs(k_chunk, 1, 3)
        m_first = jnp.maximum(m_a, qk_half(0, q_first, 1))
        wait_rows(wide, WOA0, H * D, SEM_WOA)

        m_prev, out_a = jax.lax.fori_loop(1, NH - 1, step, (m_first, jnp.zeros((8, DM), jnp.float32)))

        hl = NH - 1
        q_last = get_q(hl)
        split_pairs(v_chunk, hl, 0)
        m_a = qk_half(hl, q_last, 0)
        split_pairs(v_chunk, hl, 1)
        m_last = jnp.maximum(m_a, qk_half(hl, q_last, 1))
        split_pairs(v_chunk, hl, 2)
        for part in range(2):
            v_wait((hl - 1) % 2, part)
        acc, lsum = pv_rows(hl - 1, m_prev, 0, S // 2, zacc, zl)
        split_pairs(v_chunk, hl, 3)
        for part in range(2, 4):
            v_wait((hl - 1) % 2, part)
        acc, lsum = pv_rows(hl - 1, m_prev, S // 2, S // 2, acc, lsum)
        out_a = finish_head(hl - 1, acc, lsum, out_a)
        acc, lsum = zacc, zl
        for part in range(4):
            v_wait(hl % 2, part)
            acc, lsum = pv_rows(hl, m_last, part * VQ, VQ, acc, lsum)
        out_a = finish_head(hl, acc, lsum, out_a)
        out_ref[:, pl.ds(0, DM)] = out_a[0:NB].astype(out_ref.dtype)

    return kernel


def _make_call(NB, H, S, D, DM, DC, interpret=False):
    NH = NB * H
    bf, f32 = jnp.bfloat16, jnp.float32
    scratch = [
        pltpu.VMEM((NB, DM), bf), pltpu.VMEM((NB, DM), bf),
        pltpu.VMEM((DM, H * D), bf),
        pltpu.VMEM((DM * H, D), bf),
        pltpu.VMEM((NB * S + 2 * H * D, DM), bf),
        pltpu.VMEM((2 * DC * H + 4 * S, D), bf),
        pltpu.VMEM((2, 8, S), f32),
        pltpu.VMEM((H, S), f32),
        pltpu.VMEM((NH, D), f32),
        pltpu.VMEM((NB, DM, 128), f32),
        pltpu.VMEM((DC, 128), f32),
        pltpu.VMEM((128, DC), f32), pltpu.VMEM((128, DC), f32),
        pltpu.SemaphoreType.DMA((N_SEMS,)),
    ]
    return pl.pallas_call(
        _build_kernel(NB, H, S, D, DM, DC),
        out_shape=jax.ShapeDtypeStruct((NB, 2 * DM), bf),
        in_specs=[pl.BlockSpec(memory_space=pl.ANY)] * 11,
        out_specs=pl.BlockSpec(memory_space=pltpu.VMEM),
        scratch_shapes=scratch,
        compiler_params=pltpu.CompilerParams(vmem_limit_bytes=100 * 2**20),
        interpret=interpret,
    )


def _run(A_x, A_k_cache, A_v_cache, A_wq, A_wo, B_x, B_c_kv, B_w_q, B_w_uk, B_w_uv, B_w_o, **kw):
    NB, _, DM = A_x.shape
    _, H, S, D = A_k_cache.shape
    DC = B_c_kv.shape[2]
    NH = NB * H
    out = _make_call(NB, H, S, D, DM, DC, **kw)(
        A_x.reshape(NB, DM), A_k_cache.reshape(NH * S, D), A_v_cache.reshape(NH * S, D), A_wq, A_wo,
        B_x.reshape(NB, DM), B_c_kv.reshape(NB * S, DC),
        B_w_q.reshape(DM * H, D), B_w_uk.reshape(DC * H, D), B_w_uv.reshape(DC * H, D),
        B_w_o.reshape(H * D, DM),
    )
    return out.reshape(NB, 1, 2 * DM)


@jax.jit
def pallas_concat_heads__gqa_block_cached__compressed_kv_cla__decode_kernel(
    A_x: jax.Array,
    A_k_cache: jax.Array,
    A_v_cache: jax.Array,
    A_wq: jax.Array,
    A_wo: jax.Array,
    B_x: jax.Array,
    B_c_kv: jax.Array,
    B_w_q: jax.Array,
    B_w_uk: jax.Array,
    B_w_uv: jax.Array,
    B_w_o: jax.Array,
):
    return _run(A_x, A_k_cache, A_v_cache, A_wq, A_wo, B_x, B_c_kv, B_w_q, B_w_uk, B_w_uv, B_w_o)
```
